```python
import jax
import jax.numpy as jnp

def _softmax(x, axis=-1):
    return jax.nn.softmax(x, axis=axis)
def _gelu(x):
    return jax.nn.gelu(x, approximate=True)
def _silu(x):
    return jax.nn.silu(x)
def _sigmoid(x):
    return jax.nn.sigmoid(x)
def _layernorm(x, axis=-1, eps=1e-5):
    m = jnp.mean(x, axis=axis, keepdims=True)
    v = jnp.var(x, axis=axis, keepdims=True)
    return (x - m) / jnp.sqrt(v + eps)
def _scatter_add(tgt, idx, src, axis=0):
    return tgt.at[idx].add(src)
def _segment_sum(src, seg, n):
    return jax.ops.segment_sum(src, seg, n)
class _Rng:
    def __init__(self, key):
        self._k = key
    def _next(self):
        self._k, sub = jax.random.split(self._k)
        return sub
    def normal(self, shape):
        return jax.random.normal(self._next(), shape, dtype=jnp.bfloat16)
    def randint(self, lo, hi, shape):
        return jax.random.randint(self._next(), shape, lo, hi, dtype=jnp.int32)
    def uniform(self, shape, lo=0.0, hi=1.0):
        return jax.random.uniform(self._next(), shape, jnp.bfloat16, lo, hi)
    def permutation(self, n):
        return jax.random.permutation(self._next(), n)


kernel_name = 'parallel_sum__sliding_block_cached__mixer_s_mlp__decode'

def setup_inputs():
    _rng = _Rng(jax.random.key(int.from_bytes(__import__("os").urandom(4), "little")))
    _w = (lambda a: (lambda t: t.astype(jnp.bfloat16) if jnp.issubdtype(t.dtype, jnp.floating) else t)(jnp.asarray(a)))
    def _A_setup():
        B, Sq, D = 4, 1, 512
        Hq, Hkv, Sk, Dh = 32, 32, 8192, 128
        assert Hq % Hkv == 0, (Hq, Hkv)
        return {
            "x": _w((lambda *s: _rng.normal(s) * 0.05)(B, Sq, D)),
            "k_cache": _w((lambda *s: _rng.normal(s) * 0.05)(B, Hkv, Sk, Dh)),
            "v_cache": _w((lambda *s: _rng.normal(s) * 0.05)(B, Hkv, Sk, Dh)),
            "wq": _w((lambda *s: _rng.normal(s) * 0.05)(D, Hq * Dh) * (D ** -0.5)),
            "wo": _w((lambda *s: _rng.normal(s) * 0.05)(Hq * Dh, D) * ((Hq * Dh) ** -0.5)),
        }
    _A_in = _A_setup()

    def _B_setup():
        B, S, D, F = 4, 1, 512, 1376
        return {
            "x":  _w((lambda *s: _rng.normal(s) * 0.05)(B, S, D)),
            "w1": _w((lambda *s: _rng.normal(s) * 0.05)(D, D) * (D ** -0.5)),
            "w2": _w((lambda *s: _rng.normal(s) * 0.05)(D, D) * (D ** -0.5)),
            "w3": _w((lambda *s: _rng.normal(s) * 0.05)(D, F) * (D ** -0.5)),
            "w4": _w((lambda *s: _rng.normal(s) * 0.05)(F, D) * (F ** -0.5)),
        }
    _B_in = _B_setup()

    return {
        "A_x": _A_in["x"],
        "A_k_cache": _A_in["k_cache"],
        "A_v_cache": _A_in["v_cache"],
        "A_wq": _A_in["wq"],
        "A_wo": _A_in["wo"],
        "B_x": _B_in["x"],
        "B_w1": _B_in["w1"],
        "B_w2": _B_in["w2"],
        "B_w3": _B_in["w3"],
        "B_w4": _B_in["w4"],
    }

def reference(A_x, A_k_cache, A_v_cache, A_wq, A_wo, B_x, B_w1, B_w2, B_w3, B_w4):
    def _A_ref(x, k_cache, v_cache, wq, wo):
        B, Sq, D = x.shape
        Hq, Dh = 32, 128
        Hkv, Sk = k_cache.shape[1], k_cache.shape[2]
        W = min(4096, max(256, Sk // 4))
        rep = Hq // Hkv
        q = (lambda x, *d: x.transpose(*d))((x @ wq).reshape(B, Sq, Hq, Dh), 0, 2, 1, 3)
        k = jnp.repeat(k_cache[:, :, Sk - W:, :], rep, axis=1)
        v = jnp.repeat(v_cache[:, :, Sk - W:, :], rep, axis=1)
        scores = jnp.einsum("bhqd,bhkd->bhqk", q, k) * (Dh ** -0.5)
        p = _softmax(scores, axis=-1)
        o = jnp.einsum("bhqk,bhkd->bhqd", p, v)
        return (lambda x, *d: x.transpose(*d))(o, 0, 2, 1, 3).reshape(B, Sq, Hq * Dh) @ wo

    def _B_ref(x, w1, w2, w3, w4):
        B, S, D = x.shape
        h = _gelu(_layernorm(x, axis=-1) @ w1)
        c = D // 4
        g0 = jnp.pad(h[:, :, 0*c:1*c], ((0, 0), (1, 0), (0, 0)))[:, :S, :]
        g1 = jnp.pad(h[:, :, 1*c:2*c], ((0, 0), (0, 1), (0, 0)))[:, 1:, :]
        g2 = jnp.pad(h[:, :, 2*c:3*c], ((0, 0), (2, 0), (0, 0)))[:, :S, :]
        g3 = jnp.pad(h[:, :, 3*c:   ], ((0, 0), (0, 2), (0, 0)))[:, 2:, :]
        hs = jnp.concatenate([g0, g1, g2, g3], axis=-1) @ w2
        x1 = x + hs
        h2 = _gelu(_layernorm(x1, axis=-1) @ w3) @ w4
        return x1 + h2

    x = A_x
    xn = _layernorm(x, axis=-1)
    return x + _A_ref(xn, A_k_cache, A_v_cache, A_wq, A_wo) + _B_ref(xn, B_w1, B_w2, B_w3, B_w4)
```

```python
import functools

import jax
import jax.numpy as jnp
import jax.experimental.pallas as pl
import jax.experimental.pallas.tpu as pltpu

_EPS = 1e-5
_NSLOT = 8
_WO_CHUNKS = (1024, 1024, 1024, 512, 256, 128, 128)


def _layernorm(x):
    m = jnp.mean(x, axis=-1, keepdims=True)
    d = x - m
    v = jnp.mean(d * d, axis=-1, keepdims=True)
    return d / jnp.sqrt(v + _EPS)


def _make_kernel(B, D, H, Sk, Dh, W, F):
    N = B * H
    scale = Dh ** -0.5
    wo_starts = [sum(_WO_CHUNKS[:i]) for i in range(len(_WO_CHUNKS))]
    assert sum(_WO_CHUNKS) == H * Dh

    def kernel(x_hbm, k_hbm, v_hbm, wq_hbm, wo_hbm, w3_hbm, w4_hbm, out_ref,
               x_buf, wq_buf, wo_buf, w3_buf, w4_buf, k_buf, v_buf, q_s, o_s,
               sem_w, sem_wo, sem_k, sem_v):
        def k_copy(i, slot):
            return pltpu.make_async_copy(
                k_hbm.at[i % B, i // B, pl.ds(Sk - W, W), :], k_buf.at[slot], sem_k.at[slot])

        def v_copy(i, slot):
            return pltpu.make_async_copy(
                v_hbm.at[i % B, i // B, pl.ds(Sk - W, W), :], v_buf.at[slot], sem_v.at[slot])

        x_copy = pltpu.make_async_copy(x_hbm, x_buf, sem_w.at[0])
        wq_copy = pltpu.make_async_copy(wq_hbm, wq_buf, sem_w.at[1])
        w3_copy = pltpu.make_async_copy(w3_hbm, w3_buf, sem_w.at[2])
        w4_copy = pltpu.make_async_copy(w4_hbm, w4_buf, sem_w.at[3])
        wo_copies = [
            pltpu.make_async_copy(wo_hbm.at[pl.ds(s, c), :], wo_buf.at[pl.ds(s, c), :], sem_wo.at[j])
            for j, (s, c) in enumerate(zip(wo_starts, _WO_CHUNKS))]

        x_copy.start()
        wq_copy.start()
        for i in range(_NSLOT):
            k_copy(i, i).start()
            v_copy(i, i).start()

        x_copy.wait()
        x = jnp.concatenate(
            [x_buf[...].astype(jnp.float32), jnp.zeros((8 - B, D), jnp.float32)], axis=0)
        xn = _layernorm(x)
        xn_b = xn.astype(jnp.bfloat16)

        wq_copy.wait()
        for h in range(H):
            qh = jnp.dot(xn_b, wq_buf[:, h * Dh:(h + 1) * Dh], preferred_element_type=jnp.float32)
            q_s[h] = (qh * scale).astype(jnp.bfloat16)

        row = jax.lax.broadcasted_iota(jnp.int32, (8, Dh), 0)

        def attend(i, acc):
            slot = i % _NSLOT
            h = i // B
            b = i % B
            k_copy(i, slot).wait()
            s = jax.lax.dot_general(q_s[h], k_buf[slot], (((1,), (1,)), ((), ())),
                                    preferred_element_type=jnp.float32)
            m = jnp.max(s, axis=-1, keepdims=True)
            p = jnp.exp(s - m)
            l = jnp.sum(p, axis=-1, keepdims=True)
            v_copy(i, slot).wait()
            o = jnp.dot(p.astype(jnp.bfloat16), v_buf[slot], preferred_element_type=jnp.float32)
            o = o / l
            acc = jnp.where(row == b, o, acc)
            o_s[h] = acc.astype(jnp.bfloat16)
            return acc

        def main_body(i, acc):
            acc = attend(i, acc)
            slot = i % _NSLOT
            k_copy(i + _NSLOT, slot).start()
            v_copy(i + _NSLOT, slot).start()
            return acc

        acc0 = jnp.zeros((8, Dh), jnp.float32)
        acc = jax.lax.fori_loop(0, N - _NSLOT, main_body, acc0)

        w3_copy.start()
        w4_copy.start()
        for c in wo_copies:
            c.start()

        jax.lax.fori_loop(N - _NSLOT, N, attend, acc)

        w3_copy.wait()
        g = jax.nn.gelu(
            jax.lax.dot_general(_layernorm(xn).astype(jnp.bfloat16), w3_buf[...],
                                (((1,), (1,)), ((), ())), preferred_element_type=jnp.float32),
            approximate=True)
        w4_copy.wait()
        res = x + xn + jnp.dot(g.astype(jnp.bfloat16), w4_buf[...], preferred_element_type=jnp.float32)
        for c, s, n in zip(wo_copies, wo_starts, _WO_CHUNKS):
            c.wait()
            o_c = jnp.concatenate([o_s[h] for h in range(s // Dh, (s + n) // Dh)], axis=1)
            res = res + jnp.dot(o_c, wo_buf[pl.ds(s, n), :], preferred_element_type=jnp.float32)
        out_ref[...] = res[:B].astype(out_ref.dtype)

    return kernel


@jax.jit
def pallas_parallel_sum__sliding_block_cached__mixer_s_mlp__decode_kernel(
    A_x: jax.Array,
    A_k_cache: jax.Array,
    A_v_cache: jax.Array,
    A_wq: jax.Array,
    A_wo: jax.Array,
    B_x: jax.Array,
    B_w1: jax.Array,
    B_w2: jax.Array,
    B_w3: jax.Array,
    B_w4: jax.Array,
):
    B, Sq, D = A_x.shape
    _, H, Sk, Dh = A_k_cache.shape
    F = B_w3.shape[1]
    W = min(4096, max(256, Sk // 4))
    assert Sq == 1 and A_wq.shape == (D, H * Dh)
    bf = jnp.bfloat16
    any_spec = pl.BlockSpec(memory_space=pl.ANY)
    out = pl.pallas_call(
        _make_kernel(B, D, H, Sk, Dh, W, F),
        in_specs=[any_spec] * 7,
        out_specs=pl.BlockSpec(memory_space=pltpu.VMEM),
        out_shape=jax.ShapeDtypeStruct((B, D), A_x.dtype),
        scratch_shapes=[
            pltpu.VMEM((B, D), bf),
            pltpu.VMEM((D, H * Dh), bf),
            pltpu.VMEM((H * Dh, D), bf),
            pltpu.VMEM((F, D), bf),
            pltpu.VMEM((F, D), bf),
            pltpu.VMEM((_NSLOT, W, Dh), bf),
            pltpu.VMEM((_NSLOT, W, Dh), bf),
            pltpu.VMEM((H, 8, Dh), bf),
            pltpu.VMEM((H, 8, Dh), bf),
            pltpu.SemaphoreType.DMA((4,)),
            pltpu.SemaphoreType.DMA((len(_WO_CHUNKS),)),
            pltpu.SemaphoreType.DMA((_NSLOT,)),
            pltpu.SemaphoreType.DMA((_NSLOT,)),
        ],
        compiler_params=pltpu.CompilerParams(vmem_limit_bytes=64 * 1024 * 1024),
    )(A_x.reshape(B, D), A_k_cache, A_v_cache, A_wq, A_wo, B_w3.T, B_w4)
    return out.reshape(B, Sq, D)
```

```python
import jax
import jax.numpy as jnp
import jax.experimental.pallas as pl
import jax.experimental.pallas.tpu as pltpu

_EPS = 1e-5
_G = 8
_NG = 3
_LEAD = 19
_UP = 8
_WROWS = 32
_PRO1 = 6
_WO_A = (4, 4, 4, 4)
_WO_B = (4, 4, 4, 2, 1, 1)
_WO_LEAD = 3


def _layernorm(x):
    m = jnp.mean(x, axis=-1, keepdims=True)
    d = x - m
    v = jnp.mean(d * d, axis=-1, keepdims=True)
    return d / jnp.sqrt(v + _EPS)


def _blocks(h0, sizes):
    out = []
    for c in sizes:
        out.append((h0, c))
        h0 += c
    return out


def _make_kernel(B, D, H, Sk, Dh, W, F):
    G, NG, LEAD, UP, WROWS = _G, _NG, _LEAD, _UP, _WROWS
    NGRP = B * H // G
    ROWS = W // (2 * G * UP)
    UPG = 2 * G
    NU_KV = UPG * NGRP
    scale = Dh ** -0.5
    plan_a = _blocks(0, _WO_A)
    plan_b = _blocks(sum(_WO_A), _WO_B)
    assert sum(_WO_A) + sum(_WO_B) == H and UPG * UP * ROWS == W and F % WROWS == 0
    wo_dmas = [
        [(h0 * Dh + i * WROWS, base + bi)
         for bi, (h0, n) in enumerate(plan) for i in range(n * Dh // WROWS)]
        for plan, base in ((plan_a, 0), (plan_b, len(plan_a)))]
    NU_WO = -(-max(len(l) for l in wo_dmas) // UP)
    wo_order = []
    blk_a = list(enumerate(plan_a))
    blk_b = [(len(plan_a) + i, p) for i, p in enumerate(plan_b)]
    ia = ib = ca = cb = 0
    while ia < len(blk_a) or ib < len(blk_b):
        if ib >= len(blk_b) or (
                ia < len(blk_a) and ca + blk_a[ia][1][1] - _WO_LEAD <= cb + blk_b[ib][1][1]):
            wo_order.append(blk_a[ia]); ca += blk_a[ia][1][1]; ia += 1
        else:
            wo_order.append(blk_b[ib]); cb += blk_b[ib][1][1]; ib += 1

    def kernel(x_hbm, k_hbm, v_hbm, wq_hbm, wo_hbm, w3_hbm, w4_hbm, out_ref,
               x_buf, wq_buf, wo_buf, w3_buf, w4_buf, k_buf, v_buf, q_s, p_s, o_s,
               sem_w, sem_wo, sem_k, sem_v):

        def wait_full(buf, sem):
            pltpu.make_async_copy(buf, buf, sem).wait()

        def issue_kv(u):
            g = u // UPG
            slot = g % NG
            b = g % B
            h0 = (g // B) * G
            r0 = (u % UPG) * (UP * ROWS)
            for i in range(UP):
                r = pl.multiple_of(r0 + i * ROWS, ROWS)
                pltpu.make_async_copy(
                    k_hbm.at[b, pl.ds(h0, G), pl.ds(Sk - W + r, ROWS), :],
                    k_buf.at[slot, :, pl.ds(r, ROWS), :], sem_k.at[slot]).start(priority=0)
                pltpu.make_async_copy(
                    v_hbm.at[b, pl.ds(h0, G), pl.ds(Sk - W + r, ROWS), :],
                    v_buf.at[slot, :, pl.ds(r, ROWS), :], sem_v.at[slot]).start(priority=1)

        def issue_wo(t):
            for i in range(t * UP, (t + 1) * UP):
                for prio, lst in enumerate(wo_dmas):
                    if i < len(lst):
                        r, si = lst[i]
                        pltpu.make_async_copy(
                            wo_hbm.at[pl.ds(r, WROWS), :], wo_buf.at[pl.ds(r, WROWS), :],
                            sem_wo.at[si]).start(priority=prio)

        x_copy = pltpu.make_async_copy(x_hbm, x_buf, sem_w.at[0])
        x_copy.start()

        def wq_issue(i, c):
            half = H * Dh // 2
            for prio in range(2):
                r = pl.multiple_of((i // 2) * 8 + prio * (D // 2), 8)
                cc = pl.multiple_of((i % 2) * half, half)
                pltpu.make_async_copy(
                    wq_hbm.at[pl.ds(r, 8), pl.ds(cc, half)],
                    wq_buf.at[pl.ds(r, 8), pl.ds(cc, half)], sem_w.at[1]).start(priority=prio)
            return c
        jax.lax.fori_loop(0, D // 8, wq_issue, 0)

        x_copy.wait()
        x = jnp.concatenate(
            [x_buf[...].astype(jnp.float32), jnp.zeros((8 - B, D), jnp.float32)], axis=0)
        xn = _layernorm(x)
        xn_b = xn.astype(jnp.bfloat16)
        xnn_b = _layernorm(xn).astype(jnp.bfloat16)

        def w34_issue(i, c):
            r = pl.multiple_of(i * WROWS, WROWS)
            pltpu.make_async_copy(w3_hbm.at[pl.ds(r, WROWS), :], w3_buf.at[pl.ds(r, WROWS), :],
                                  sem_w.at[2]).start(priority=0)
            pltpu.make_async_copy(w4_hbm.at[pl.ds(r, WROWS), :], w4_buf.at[pl.ds(r, WROWS), :],
                                  sem_w.at[3]).start(priority=1)
            return c
        jax.lax.fori_loop(0, F // WROWS, w34_issue, 0)

        wait_full(wq_buf, sem_w.at[1])
        for h in range(H):
            qh = jnp.dot(xn_b, wq_buf[:, h * Dh:(h + 1) * Dh], preferred_element_type=jnp.float32)
            q_s[h] = (qh * scale).astype(jnp.bfloat16)
            o_s[h] = jnp.zeros((8, Dh), jnp.float32)

        def kv_prologue(u, c):
            issue_kv(u)
            return c
        jax.lax.fori_loop(0, _PRO1, kv_prologue, 0)

        wait_full(w3_buf, sem_w.at[2])
        wait_full(w4_buf, sem_w.at[3])
        hid = jax.nn.gelu(
            jax.lax.dot_general(xnn_b, w3_buf[...], (((1,), (1,)), ((), ())),
                                preferred_element_type=jnp.float32),
            approximate=True)
        res = x + xn + jnp.dot(hid.astype(jnp.bfloat16), w4_buf[...],
                               preferred_element_type=jnp.float32)

        jax.lax.fori_loop(_PRO1, LEAD, kv_prologue, 0)

        row = jax.lax.broadcasted_iota(jnp.int32, (8, Dh), 0)

        def scores(slot, h0, k):
            s = jax.lax.dot_general(q_s[h0 + k], k_buf[slot, k], (((1,), (1,)), ((), ())),
                                    preferred_element_type=jnp.float32)
            m = jnp.max(s, axis=-1, keepdims=True)
            p = jnp.exp(s - m)
            l = jnp.sum(p, axis=-1, keepdims=True)
            p_s[k] = (p * (1.0 / l)).astype(jnp.bfloat16)

        def values(slot, b, h0, k):
            o = jnp.dot(p_s[k], v_buf[slot, k], preferred_element_type=jnp.float32)
            o_s[h0 + k] = jnp.where(row == b, o, o_s[h0 + k])

        wo_main = max(0, min(NU_WO, UPG * (NGRP - 1) + LEAD - NU_KV))

        def issue(u):
            @pl.when(u < NU_KV)
            def _():
                issue_kv(u)
            for t in range(wo_main):
                @pl.when(u == NU_KV + t)
                def _():
                    issue_wo(t)

        def group(g, carry):
            slot = g % NG
            b = g % B
            h0 = (g // B) * G

            def step1(k, c):
                issue(g * UPG + k + LEAD)
                @pl.when(k == 0)
                def _():
                    wait_full(k_buf.at[slot], sem_k.at[slot])
                scores(slot, h0, k)
                return c
            jax.lax.fori_loop(0, G, step1, 0)

            def step2(k, c):
                issue(g * UPG + G + k + LEAD)
                @pl.when(k == 0)
                def _():
                    wait_full(v_buf.at[slot], sem_v.at[slot])
                values(slot, b, h0, k)
                return c
            jax.lax.fori_loop(0, G, step2, 0)
            return carry

        jax.lax.fori_loop(0, NGRP - 1, group, 0)

        gl = NGRP - 1
        slot, b, h0 = gl % NG, gl % B, (gl // B) * G
        first = UPG * gl + LEAD
        assert first >= NU_KV
        rest = [u - NU_KV for u in range(first, NU_KV + NU_WO)]
        for t in rest[:1]:
            issue_wo(t)
        wait_full(k_buf.at[slot], sem_k.at[slot])

        def last1(k, c):
            scores(slot, h0, k)
            return c
        jax.lax.fori_loop(0, G, last1, 0, unroll=4)
        for t in rest[1:]:
            issue_wo(t)
        wait_full(v_buf.at[slot], sem_v.at[slot])

        def last2(k, c):
            values(slot, b, h0, k)
            return c
        jax.lax.fori_loop(0, G, last2, 0, unroll=4)

        for si, (hh, n) in wo_order:
            blk = wo_buf.at[pl.ds(hh * Dh, n * Dh), :]
            wait_full(blk, sem_wo.at[si])
            o_c = jnp.concatenate([o_s[hh + i] for i in range(n)], axis=1).astype(jnp.bfloat16)
            res = res + jnp.dot(o_c, blk[...], preferred_element_type=jnp.float32)
        out_ref[...] = res[:B].astype(out_ref.dtype)

    return kernel, len(plan_a) + len(plan_b)


@jax.jit
def pallas_parallel_sum__sliding_block_cached__mixer_s_mlp__decode_kernel(
    A_x: jax.Array,
    A_k_cache: jax.Array,
    A_v_cache: jax.Array,
    A_wq: jax.Array,
    A_wo: jax.Array,
    B_x: jax.Array,
    B_w1: jax.Array,
    B_w2: jax.Array,
    B_w3: jax.Array,
    B_w4: jax.Array,
):
    B, Sq, D = A_x.shape
    _, H, Sk, Dh = A_k_cache.shape
    F = B_w3.shape[1]
    W = min(4096, max(256, Sk // 4))
    assert Sq == 1 and A_wq.shape == (D, H * Dh)
    bf = jnp.bfloat16
    kernel, n_wo_sems = _make_kernel(B, D, H, Sk, Dh, W, F)
    out = pl.pallas_call(
        kernel,
        in_specs=[pl.BlockSpec(memory_space=pl.ANY)] * 7,
        out_specs=pl.BlockSpec(memory_space=pltpu.VMEM),
        out_shape=jax.ShapeDtypeStruct((B, D), A_x.dtype),
        scratch_shapes=[
            pltpu.VMEM((B, D), bf),
            pltpu.VMEM((D, H * Dh), bf),
            pltpu.VMEM((H * Dh, D), bf),
            pltpu.VMEM((F, D), bf),
            pltpu.VMEM((F, D), bf),
            pltpu.VMEM((_NG, _G, W, Dh), bf),
            pltpu.VMEM((_NG, _G, W, Dh), bf),
            pltpu.VMEM((H, 8, Dh), bf),
            pltpu.VMEM((_G, 8, W), bf),
            pltpu.VMEM((H, 8, Dh), jnp.float32),
            pltpu.SemaphoreType.DMA((4,)),
            pltpu.SemaphoreType.DMA((n_wo_sems,)),
            pltpu.SemaphoreType.DMA((_NG,)),
            pltpu.SemaphoreType.DMA((_NG,)),
        ],
        compiler_params=pltpu.CompilerParams(
            vmem_limit_bytes=64 * 1024 * 1024,
            disable_bounds_checks=True,
            disable_semaphore_checks=True,
        ),
    )(A_x.reshape(B, D), A_k_cache, A_v_cache, A_wq, A_wo, B_w3.T, B_w4)
    return out.reshape(B, Sq, D)
```

```python
import jax
import jax.numpy as jnp
import jax.experimental.pallas as pl
import jax.experimental.pallas.tpu as pltpu

_EPS = 1e-5
_G = 8
_NG = 3
_LEAD = 19
_UP = 8
_VOFF = 24
_PRO1 = 12
_WQ_SEG = 4
_WROWS = 16
_WO_A = (256, 256, 256, 256)
_WO_B = (256, 256, 256, 128, 64, 64)
_WO_LEAD = 384


def _layernorm(x):
    m = jnp.mean(x, axis=-1, keepdims=True)
    d = x - m
    v = jnp.mean(d * d, axis=-1, keepdims=True)
    return d / jnp.sqrt(v + _EPS)


def _blocks(r0, sizes):
    out = []
    for n in sizes:
        out.append((r0, n))
        r0 += n
    return out


def _make_kernel(B, D, H, Sk, Dh, W, F):
    G, NG, LEAD, UP, WROWS = _G, _NG, _LEAD, _UP, _WROWS
    NGRP = B * H // G
    ROWS = W // (2 * G * UP)
    UPG = 2 * G
    NU_KV = UPG * NGRP
    HALF = H * Dh // 2
    scale = Dh ** -0.5
    plan_a = _blocks(0, _WO_A)
    plan_b = _blocks(sum(_WO_A), _WO_B)
    assert sum(_WO_A) + sum(_WO_B) == HALF and UPG * UP * ROWS == W and (F // 2) % WROWS == 0
    wo_dmas = [
        [(r0 + i * WROWS, base + bi) for bi, (r0, n) in enumerate(plan) for i in range(n // WROWS)]
        for plan, base in ((plan_a, 0), (plan_b, len(plan_a)))]
    NU_WO = -(-max(len(l) for l in wo_dmas) // UP)
    wo_order = []
    blk_a = list(enumerate(plan_a))
    blk_b = [(len(plan_a) + i, p) for i, p in enumerate(plan_b)]
    ia = ib = ca = cb = 0
    while ia < len(blk_a) or ib < len(blk_b):
        if ib >= len(blk_b) or (
                ia < len(blk_a) and ca + blk_a[ia][1][1] - _WO_LEAD <= cb + blk_b[ib][1][1]):
            wo_order.append(blk_a[ia]); ca += blk_a[ia][1][1]; ia += 1
        else:
            wo_order.append(blk_b[ib]); cb += blk_b[ib][1][1]; ib += 1

    def kernel(x_hbm, k_hbm, v_hbm, wq_hbm, wo_hbm, w3_hbm, w4_hbm, out_ref,
               x_buf, wq_buf, wo_buf, w3_buf, w4_buf, k_buf, v_buf, q_s, p_s, o_s,
               sem_w, sem_wo, sem_k, sem_v):

        def wait_full(buf, sem):
            pltpu.make_async_copy(buf, buf, sem).wait()

        def issue_kv(u):
            g = u // UPG
            slot = g % NG
            b = g % B
            h0 = (g // B) * G
            r0 = (u % UPG) * (UP * ROWS)
            for i in range(UP):
                rk = pl.multiple_of(r0 + i * ROWS, ROWS)
                rv = pl.multiple_of((rk + _VOFF * ROWS) % W, ROWS)
                pltpu.make_async_copy(
                    k_hbm.at[b, pl.ds(h0, G), pl.ds(Sk - W + rk, ROWS), :],
                    k_buf.at[slot, :, pl.ds(rk, ROWS), :], sem_k.at[slot]).start(priority=0)
                pltpu.make_async_copy(
                    v_hbm.at[b, pl.ds(h0, G), pl.ds(Sk - W + rv, ROWS), :],
                    v_buf.at[slot, :, pl.ds(rv, ROWS), :], sem_v.at[slot]).start(priority=1)

        def issue_wo(t):
            for i in range(t * UP, (t + 1) * UP):
                for prio, lst in enumerate(wo_dmas):
                    if i < len(lst):
                        r, si = lst[i]
                        pltpu.make_async_copy(
                            wo_hbm.at[:, pl.ds(r, WROWS), :], wo_buf.at[:, pl.ds(r, WROWS), :],
                            sem_wo.at[si]).start(priority=prio)

        x_copy = pltpu.make_async_copy(x_hbm, x_buf, sem_w.at[0])
        x_copy.start()

        WQC = 512
        ncb = H * Dh // WQC
        n_wq = (D // _WQ_SEG // 8) * ncb

        def wq_issue(i, c):
            for prio in range(2):
                d = i + prio * (n_wq // 2)
                r = pl.multiple_of((d // ncb) * 8, 8)
                cc = pl.multiple_of((d % ncb) * WQC, WQC)
                pltpu.make_async_copy(
                    wq_hbm.at[:, pl.ds(r, 8), pl.ds(cc, WQC)],
                    wq_buf.at[:, pl.ds(r, 8), pl.ds(cc, WQC)], sem_w.at[1]).start(priority=prio)
            return c
        jax.lax.fori_loop(0, n_wq // 2, wq_issue, 0)

        x_copy.wait()
        x = jnp.concatenate(
            [x_buf[...].astype(jnp.float32), jnp.zeros((8 - B, D), jnp.float32)], axis=0)
        xn = _layernorm(x)
        xn_b = xn.astype(jnp.bfloat16)
        xnn_b = _layernorm(xn).astype(jnp.bfloat16)

        def w34_issue(i, c):
            r = pl.multiple_of(i * WROWS, WROWS)
            pltpu.make_async_copy(w3_hbm.at[:, pl.ds(r, WROWS), :], w3_buf.at[:, pl.ds(r, WROWS), :],
                                  sem_w.at[2]).start(priority=0)
            pltpu.make_async_copy(w4_hbm.at[:, pl.ds(r, WROWS), :], w4_buf.at[:, pl.ds(r, WROWS), :],
                                  sem_w.at[3]).start(priority=1)
            return c
        jax.lax.fori_loop(0, F // 2 // WROWS, w34_issue, 0)

        wait_full(wq_buf, sem_w.at[1])
        for h in range(H):
            wq_h = wq_buf[:, :, h * Dh:(h + 1) * Dh].reshape(D, Dh)
            qh = jnp.dot(xn_b, wq_h, preferred_element_type=jnp.float32)
            q_s[h] = (qh * scale).astype(jnp.bfloat16)
            o_s[h] = jnp.zeros((8, Dh), jnp.float32)

        def kv_prologue(u, c):
            issue_kv(u)
            return c
        jax.lax.fori_loop(0, _PRO1, kv_prologue, 0)

        wait_full(w3_buf, sem_w.at[2])
        wait_full(w4_buf, sem_w.at[3])
        hid = jax.nn.gelu(
            jax.lax.dot_general(xnn_b, w3_buf[...].reshape(F, D), (((1,), (1,)), ((), ())),
                                preferred_element_type=jnp.float32),
            approximate=True)
        res = x + xn + jnp.dot(hid.astype(jnp.bfloat16), w4_buf[...].reshape(F, D),
                               preferred_element_type=jnp.float32)

        jax.lax.fori_loop(_PRO1, LEAD, kv_prologue, 0)

        row = jax.lax.broadcasted_iota(jnp.int32, (8, Dh), 0)

        def scores(slot, h0, k):
            s = jax.lax.dot_general(q_s[h0 + k], k_buf[slot, k], (((1,), (1,)), ((), ())),
                                    preferred_element_type=jnp.float32)
            m = jnp.max(s, axis=-1, keepdims=True)
            p = jnp.exp(s - m)
            l = jnp.sum(p, axis=-1, keepdims=True)
            p_s[k] = (p * (1.0 / l)).astype(jnp.bfloat16)

        def values(slot, b, h0, k):
            o = jnp.dot(p_s[k], v_buf[slot, k], preferred_element_type=jnp.float32)
            o_s[h0 + k] = jnp.where(row == b, o, o_s[h0 + k])

        wo_main = max(0, min(NU_WO, UPG * (NGRP - 1) + LEAD - NU_KV))

        def issue(u):
            @pl.when(u < NU_KV)
            def _():
                issue_kv(u)
            for t in range(wo_main):
                @pl.when(u == NU_KV + t)
                def _():
                    issue_wo(t)

        def group(g, carry):
            slot = g % NG
            b = g % B
            h0 = (g // B) * G

            def step1(k, c):
                issue(g * UPG + k + LEAD)
                @pl.when(k == 0)
                def _():
                    wait_full(k_buf.at[slot], sem_k.at[slot])
                scores(slot, h0, k)
                return c
            jax.lax.fori_loop(0, G, step1, 0)

            def step2(k, c):
                issue(g * UPG + G + k + LEAD)
                @pl.when(k == 0)
                def _():
                    wait_full(v_buf.at[slot], sem_v.at[slot])
                values(slot, b, h0, k)
                return c
            jax.lax.fori_loop(0, G, step2, 0)
            return carry

        jax.lax.fori_loop(0, NGRP - 1, group, 0)

        gl = NGRP - 1
        slot, b, h0 = gl % NG, gl % B, (gl // B) * G
        first = UPG * gl + LEAD
        assert first >= NU_KV
        rest = [u - NU_KV for u in range(first, NU_KV + NU_WO)]
        for t in rest[:1]:
            issue_wo(t)
        wait_full(k_buf.at[slot], sem_k.at[slot])

        def last1(k, c):
            scores(slot, h0, k)
            return c
        jax.lax.fori_loop(0, G, last1, 0, unroll=4)
        for t in rest[1:3]:
            issue_wo(t)
        wait_full(v_buf.at[slot], sem_v.at[slot])
        for t in rest[3:]:
            issue_wo(t)

        def last2(k, c):
            values(slot, b, h0, k)
            return c
        jax.lax.fori_loop(0, G, last2, 0, unroll=4)

        def o_cols(start, n):
            parts, pos = [], start
            while pos < start + n:
                h, d0 = divmod(pos, Dh)
                take = min(Dh - d0, start + n - pos)
                parts.append(o_s[h][:, d0:d0 + take])
                pos += take
            return parts

        for si, (r0, n) in wo_order:
            blk = wo_buf.at[:, pl.ds(r0, n), :]
            o_c = jnp.concatenate(o_cols(r0, n) + o_cols(HALF + r0, n), axis=1).astype(jnp.bfloat16)
            wait_full(blk, sem_wo.at[si])
            res = res + jnp.dot(o_c, blk[...].reshape(2 * n, D), preferred_element_type=jnp.float32)
        out_ref[...] = res[:B].astype(out_ref.dtype)

    return kernel, len(plan_a) + len(plan_b)


@jax.jit
def pallas_parallel_sum__sliding_block_cached__mixer_s_mlp__decode_kernel(
    A_x: jax.Array,
    A_k_cache: jax.Array,
    A_v_cache: jax.Array,
    A_wq: jax.Array,
    A_wo: jax.Array,
    B_x: jax.Array,
    B_w1: jax.Array,
    B_w2: jax.Array,
    B_w3: jax.Array,
    B_w4: jax.Array,
):
    B, Sq, D = A_x.shape
    _, H, Sk, Dh = A_k_cache.shape
    F = B_w3.shape[1]
    W = min(4096, max(256, Sk // 4))
    assert Sq == 1 and A_wq.shape == (D, H * Dh)
    bf = jnp.bfloat16
    kernel, n_wo_sems = _make_kernel(B, D, H, Sk, Dh, W, F)
    out = pl.pallas_call(
        kernel,
        in_specs=[pl.BlockSpec(memory_space=pl.ANY)] * 7,
        out_specs=pl.BlockSpec(memory_space=pltpu.VMEM),
        out_shape=jax.ShapeDtypeStruct((B, D), A_x.dtype),
        scratch_shapes=[
            pltpu.VMEM((B, D), bf),
            pltpu.VMEM((_WQ_SEG, D // _WQ_SEG, H * Dh), bf),
            pltpu.VMEM((2, H * Dh // 2, D), bf),
            pltpu.VMEM((2, F // 2, D), bf),
            pltpu.VMEM((2, F // 2, D), bf),
            pltpu.VMEM((_NG, _G, W, Dh), bf),
            pltpu.VMEM((_NG, _G, W, Dh), bf),
            pltpu.VMEM((H, 8, Dh), bf),
            pltpu.VMEM((_G, 8, W), bf),
            pltpu.VMEM((H, 8, Dh), jnp.float32),
            pltpu.SemaphoreType.DMA((4,)),
            pltpu.SemaphoreType.DMA((n_wo_sems,)),
            pltpu.SemaphoreType.DMA((_NG,)),
            pltpu.SemaphoreType.DMA((_NG,)),
        ],
        compiler_params=pltpu.CompilerParams(
            vmem_limit_bytes=64 * 1024 * 1024,
            disable_bounds_checks=True,
            disable_semaphore_checks=True,
        ),
    )(A_x.reshape(B, D), A_k_cache, A_v_cache,
      A_wq.reshape(_WQ_SEG, D // _WQ_SEG, H * Dh), A_wo.reshape(2, H * Dh // 2, D),
      B_w3.T.reshape(2, F // 2, D), B_w4.reshape(2, F // 2, D))
    return out.reshape(B, Sq, D)
```

```python
import jax
import jax.numpy as jnp
import jax.experimental.pallas as pl
import jax.experimental.pallas.tpu as pltpu

_EPS = 1e-5
_G = 8
_NG = 3
_LEAD = 19
_UP = 8
_VOFF = 24
_PRO1 = 12
_WQ_SEG = 4
_WQ_HEAD = 32
_WROWS = 16
_WO_A = (256, 256, 256, 256)
_WO_B = (256, 256, 256, 128, 64, 64)
_WO_LEAD = 384


def _layernorm(x):
    m = jnp.mean(x, axis=-1, keepdims=True)
    d = x - m
    v = jnp.mean(d * d, axis=-1, keepdims=True)
    return d / jnp.sqrt(v + _EPS)


def _blocks(r0, sizes):
    out = []
    for n in sizes:
        out.append((r0, n))
        r0 += n
    return out


def _make_kernel(B, D, H, Sk, Dh, W, F):
    G, NG, LEAD, UP, WROWS = _G, _NG, _LEAD, _UP, _WROWS
    NGRP = B * H // G
    ROWS = W // (2 * G * UP)
    UPG = 2 * G
    NU_KV = UPG * NGRP
    HALF = H * Dh // 2
    scale = Dh ** -0.5
    plan_a = _blocks(0, _WO_A)
    plan_b = _blocks(sum(_WO_A), _WO_B)
    assert sum(_WO_A) + sum(_WO_B) == HALF and UPG * UP * ROWS == W and (F // 2) % WROWS == 0
    wo_dmas = [
        [(r0 + i * WROWS, base + bi) for bi, (r0, n) in enumerate(plan) for i in range(n // WROWS)]
        for plan, base in ((plan_a, 0), (plan_b, len(plan_a)))]
    NU_WO = -(-max(len(l) for l in wo_dmas) // UP)
    wo_order = []
    blk_a = list(enumerate(plan_a))
    blk_b = [(len(plan_a) + i, p) for i, p in enumerate(plan_b)]
    ia = ib = ca = cb = 0
    while ia < len(blk_a) or ib < len(blk_b):
        if ib >= len(blk_b) or (
                ia < len(blk_a) and ca + blk_a[ia][1][1] - _WO_LEAD <= cb + blk_b[ib][1][1]):
            wo_order.append(blk_a[ia]); ca += blk_a[ia][1][1]; ia += 1
        else:
            wo_order.append(blk_b[ib]); cb += blk_b[ib][1][1]; ib += 1

    def kernel(x_hbm, k_hbm, v_hbm, wq_hbm, wo_hbm, w3_hbm, w4_hbm, out_ref,
               x_buf, wq_buf, wo_buf, w3_buf, w4_buf, k_buf, v_buf, q_s, p_s, o_s,
               sem_w, sem_wo, sem_k, sem_v):

        def wait_full(buf, sem):
            pltpu.make_async_copy(buf, buf, sem).wait()

        def issue_kv(u):
            g = u // UPG
            slot = g % NG
            b = g % B
            h0 = (g // B) * G
            r0 = (u % UPG) * (UP * ROWS)
            for i in range(UP):
                rk = pl.multiple_of(r0 + i * ROWS, ROWS)
                rv = pl.multiple_of((rk + _VOFF * ROWS) % W, ROWS)
                pltpu.make_async_copy(
                    k_hbm.at[b, pl.ds(h0, G), pl.ds(Sk - W + rk, ROWS), :],
                    k_buf.at[slot, :, pl.ds(rk, ROWS), :], sem_k.at[slot]).start(priority=0)
                pltpu.make_async_copy(
                    v_hbm.at[b, pl.ds(h0, G), pl.ds(Sk - W + rv, ROWS), :],
                    v_buf.at[slot, :, pl.ds(rv, ROWS), :], sem_v.at[slot]).start(priority=1)

        def issue_wo(t):
            for i in range(t * UP, (t + 1) * UP):
                for prio, lst in enumerate(wo_dmas):
                    if i < len(lst):
                        r, si = lst[i]
                        pltpu.make_async_copy(
                            wo_hbm.at[:, pl.ds(r, WROWS), :], wo_buf.at[:, pl.ds(r, WROWS), :],
                            sem_wo.at[si]).start(priority=prio)

        x_copy = pltpu.make_async_copy(x_hbm, x_buf, sem_w.at[0])
        x_copy.start()

        WQC = 512
        ncb = H * Dh // WQC
        n_wq = (D // _WQ_SEG // 8) * ncb
        n_wq0 = (n_wq - _WQ_HEAD) // 2

        def wq_start(d, prio):
            r = pl.multiple_of((d // ncb) * 8, 8)
            cc = pl.multiple_of((d % ncb) * WQC, WQC)
            pltpu.make_async_copy(
                wq_hbm.at[:, pl.ds(r, 8), pl.ds(cc, WQC)],
                wq_buf.at[:, pl.ds(r, 8), pl.ds(cc, WQC)], sem_w.at[1]).start(priority=prio)

        def wq_head(i, c):
            wq_start(n_wq0 + i, 1)
            return c
        jax.lax.fori_loop(0, _WQ_HEAD, wq_head, 0, unroll=True)

        def wq_issue(i, c):
            wq_start(i, 0)
            wq_start(n_wq0 + _WQ_HEAD + i, 1)
            return c
        jax.lax.fori_loop(0, n_wq0, wq_issue, 0, unroll=8)

        x_copy.wait()
        x = jnp.concatenate(
            [x_buf[...].astype(jnp.float32), jnp.zeros((8 - B, D), jnp.float32)], axis=0)
        xn = _layernorm(x)
        xn_b = xn.astype(jnp.bfloat16)
        xnn_b = _layernorm(xn).astype(jnp.bfloat16)

        def w34_issue(i, c):
            r = pl.multiple_of(i * WROWS, WROWS)
            pltpu.make_async_copy(w3_hbm.at[:, pl.ds(r, WROWS), :], w3_buf.at[:, pl.ds(r, WROWS), :],
                                  sem_w.at[2]).start(priority=0)
            pltpu.make_async_copy(w4_hbm.at[:, pl.ds(r, WROWS), :], w4_buf.at[:, pl.ds(r, WROWS), :],
                                  sem_w.at[3]).start(priority=1)
            return c
        jax.lax.fori_loop(0, F // 2 // WROWS, w34_issue, 0)

        wait_full(wq_buf, sem_w.at[1])
        for h in range(H):
            wq_h = wq_buf[:, :, h * Dh:(h + 1) * Dh].reshape(D, Dh)
            qh = jnp.dot(xn_b, wq_h, preferred_element_type=jnp.float32)
            q_s[h] = (qh * scale).astype(jnp.bfloat16)
            o_s[h] = jnp.zeros((8, Dh), jnp.float32)

        def kv_prologue(u, c):
            issue_kv(u)
            return c
        jax.lax.fori_loop(0, _PRO1, kv_prologue, 0)

        wait_full(w3_buf, sem_w.at[2])
        wait_full(w4_buf, sem_w.at[3])
        hid = jax.nn.gelu(
            jax.lax.dot_general(xnn_b, w3_buf[...].reshape(F, D), (((1,), (1,)), ((), ())),
                                preferred_element_type=jnp.float32),
            approximate=True)
        res = x + xn + jnp.dot(hid.astype(jnp.bfloat16), w4_buf[...].reshape(F, D),
                               preferred_element_type=jnp.float32)

        jax.lax.fori_loop(_PRO1, LEAD, kv_prologue, 0)

        row = jax.lax.broadcasted_iota(jnp.int32, (8, Dh), 0)

        def scores(slot, h0, k):
            s = jax.lax.dot_general(q_s[h0 + k], k_buf[slot, k], (((1,), (1,)), ((), ())),
                                    preferred_element_type=jnp.float32)
            m = jnp.max(s, axis=-1, keepdims=True)
            p = jnp.exp(s - m)
            l = jnp.sum(p, axis=-1, keepdims=True)
            p_s[k] = (p * (1.0 / l)).astype(jnp.bfloat16)

        def values(slot, b, h0, k):
            o = jnp.dot(p_s[k], v_buf[slot, k], preferred_element_type=jnp.float32)
            o_s[h0 + k] = jnp.where(row == b, o, o_s[h0 + k])

        wo_main = max(0, min(NU_WO, UPG * (NGRP - 1) + LEAD - NU_KV))

        def issue(u):
            @pl.when(u < NU_KV)
            def _():
                issue_kv(u)
            for t in range(wo_main):
                @pl.when(u == NU_KV + t)
                def _():
                    issue_wo(t)

        def group(g, carry):
            slot = g % NG
            b = g % B
            h0 = (g // B) * G

            def step1(k, c):
                issue(g * UPG + k + LEAD)
                @pl.when(k == 0)
                def _():
                    wait_full(k_buf.at[slot], sem_k.at[slot])
                scores(slot, h0, k)
                return c
            jax.lax.fori_loop(0, G, step1, 0)

            def step2(k, c):
                issue(g * UPG + G + k + LEAD)
                @pl.when(k == 0)
                def _():
                    wait_full(v_buf.at[slot], sem_v.at[slot])
                values(slot, b, h0, k)
                return c
            jax.lax.fori_loop(0, G, step2, 0)
            return carry

        jax.lax.fori_loop(0, NGRP - 1, group, 0)

        gl = NGRP - 1
        slot, b, h0 = gl % NG, gl % B, (gl // B) * G
        first = UPG * gl + LEAD
        assert first >= NU_KV
        rest = [u - NU_KV for u in range(first, NU_KV + NU_WO)]
        for t in rest[:1]:
            issue_wo(t)
        wait_full(k_buf.at[slot], sem_k.at[slot])

        def last1(k, c):
            scores(slot, h0, k)
            return c
        jax.lax.fori_loop(0, G, last1, 0, unroll=4)
        for t in rest[1:3]:
            issue_wo(t)
        wait_full(v_buf.at[slot], sem_v.at[slot])
        for t in rest[3:]:
            issue_wo(t)

        def last2(k, c):
            values(slot, b, h0, k)
            return c
        jax.lax.fori_loop(0, G, last2, 0, unroll=4)

        def o_cols(start, n):
            parts, pos = [], start
            while pos < start + n:
                h, d0 = divmod(pos, Dh)
                take = min(Dh - d0, start + n - pos)
                parts.append(o_s[h][:, d0:d0 + take])
                pos += take
            return parts

        for si, (r0, n) in wo_order:
            blk = wo_buf.at[:, pl.ds(r0, n), :]
            o_c = jnp.concatenate(o_cols(r0, n) + o_cols(HALF + r0, n), axis=1).astype(jnp.bfloat16)
            wait_full(blk, sem_wo.at[si])
            res = res + jnp.dot(o_c, blk[...].reshape(2 * n, D), preferred_element_type=jnp.float32)
        out_ref[...] = res[:B].astype(out_ref.dtype)

    return kernel, len(plan_a) + len(plan_b)


@jax.jit
def pallas_parallel_sum__sliding_block_cached__mixer_s_mlp__decode_kernel(
    A_x: jax.Array,
    A_k_cache: jax.Array,
    A_v_cache: jax.Array,
    A_wq: jax.Array,
    A_wo: jax.Array,
    B_x: jax.Array,
    B_w1: jax.Array,
    B_w2: jax.Array,
    B_w3: jax.Array,
    B_w4: jax.Array,
):
    B, Sq, D = A_x.shape
    _, H, Sk, Dh = A_k_cache.shape
    F = B_w3.shape[1]
    W = min(4096, max(256, Sk // 4))
    assert Sq == 1 and A_wq.shape == (D, H * Dh)
    bf = jnp.bfloat16
    kernel, n_wo_sems = _make_kernel(B, D, H, Sk, Dh, W, F)
    out = pl.pallas_call(
        kernel,
        in_specs=[pl.BlockSpec(memory_space=pl.ANY)] * 7,
        out_specs=pl.BlockSpec(memory_space=pltpu.VMEM),
        out_shape=jax.ShapeDtypeStruct((B, D), A_x.dtype),
        scratch_shapes=[
            pltpu.VMEM((B, D), bf),
            pltpu.VMEM((_WQ_SEG, D // _WQ_SEG, H * Dh), bf),
            pltpu.VMEM((2, H * Dh // 2, D), bf),
            pltpu.VMEM((2, F // 2, D), bf),
            pltpu.VMEM((2, F // 2, D), bf),
            pltpu.VMEM((_NG, _G, W, Dh), bf),
            pltpu.VMEM((_NG, _G, W, Dh), bf),
            pltpu.VMEM((H, 8, Dh), bf),
            pltpu.VMEM((_G, 8, W), bf),
            pltpu.VMEM((H, 8, Dh), jnp.float32),
            pltpu.SemaphoreType.DMA((4,)),
            pltpu.SemaphoreType.DMA((n_wo_sems,)),
            pltpu.SemaphoreType.DMA((_NG,)),
            pltpu.SemaphoreType.DMA((_NG,)),
        ],
        compiler_params=pltpu.CompilerParams(
            vmem_limit_bytes=64 * 1024 * 1024,
            disable_bounds_checks=True,
            disable_semaphore_checks=True,
        ),
    )(A_x.reshape(B, D), A_k_cache, A_v_cache,
      A_wq.reshape(_WQ_SEG, D // _WQ_SEG, H * Dh), A_wo.reshape(2, H * Dh // 2, D),
      B_w3.T.reshape(2, F // 2, D), B_w4.reshape(2, F // 2, D))
    return out.reshape(B, Sq, D)
```
